```python
import jax
import jax.numpy as jnp

def _softmax(x, axis=-1):
    return jax.nn.softmax(x, axis=axis)

def _gelu(x):
    return jax.nn.gelu(x, approximate=True)

def _silu(x):
    return jax.nn.silu(x)

def _sigmoid(x):
    return jax.nn.sigmoid(x)

def _layernorm(x, axis=-1, eps=1e-05):
    m = jnp.mean(x, axis=axis, keepdims=True)
    v = jnp.var(x, axis=axis, keepdims=True)
    return (x - m) / jnp.sqrt(v + eps)

def _scatter_add(tgt, idx, src, axis=0):
    return tgt.at[idx].add(src)

def _segment_sum(src, seg, n):
    return jax.ops.segment_sum(src, seg, n)

class _Rng:

    def __init__(self, key):
        self._k = key

    def _next(self):
        self._k, sub = jax.random.split(self._k)
        return sub

    def normal(self, shape):
        return jax.random.normal(self._next(), shape, dtype=jnp.bfloat16)

    def randint(self, lo, hi, shape):
        return jax.random.randint(self._next(), shape, lo, hi, dtype=jnp.int32)

    def uniform(self, shape, lo=0.0, hi=1.0):
        return jax.random.uniform(self._next(), shape, jnp.bfloat16, lo, hi)

    def permutation(self, n):
        return jax.random.permutation(self._next(), n)
kernel_name = 'adaLN_cond__sliding_block_cached__glu_gated_glu__decode'

def setup_inputs():
    _rng = _Rng(jax.random.key(int.from_bytes(__import__("os").urandom(4), "little")))
    _w = lambda a: (lambda t: t.astype(jnp.bfloat16) if jnp.issubdtype(t.dtype, jnp.floating) else t)(jnp.asarray(a))

    def _A_setup():
        B, Sq, D = (8, 1, 512)
        Hq, Hkv, Sk, Dh = (32, 32, 4096, 128)
        assert Hq % Hkv == 0, (Hq, Hkv)
        return {'x': _w((lambda *s: _rng.normal(s) * 0.05)(B, Sq, D)), 'k_cache': _w((lambda *s: _rng.normal(s) * 0.05)(B, Hkv, Sk, Dh)), 'v_cache': _w((lambda *s: _rng.normal(s) * 0.05)(B, Hkv, Sk, Dh)), 'wq': _w((lambda *s: _rng.normal(s) * 0.05)(D, Hq * Dh) * D ** (-0.5)), 'wo': _w((lambda *s: _rng.normal(s) * 0.05)(Hq * Dh, D) * (Hq * Dh) ** (-0.5))}
    _A_in = _A_setup()

    def _B_setup():
        B, S, D, F = (8, 1, 512, 1376)
        return {'x': _w((lambda *s: _rng.normal(s) * 0.05)(B, S, D)), 'w_gate': _w((lambda *s: _rng.normal(s) * 0.05)(D, F)), 'w_up': _w((lambda *s: _rng.normal(s) * 0.05)(D, F)), 'w_down': _w((lambda *s: _rng.normal(s) * 0.05)(F, D))}
    _B_in = _B_setup()
    return {'A_x': _A_in['x'], 'A_k_cache': _A_in['k_cache'], 'A_v_cache': _A_in['v_cache'], 'A_wq': _A_in['wq'], 'A_wo': _A_in['wo'], 'B_x': _B_in['x'], 'B_w_gate': _B_in['w_gate'], 'B_w_up': _B_in['w_up'], 'B_w_down': _B_in['w_down'], 'c': _w((lambda *s: _rng.normal(s) * 0.05)(8, 512)), 'w_mod': _w((lambda *s: _rng.normal(s) * 0.05)(512, 6 * 512) * 512 ** (-0.5))}

def reference(A_x, A_k_cache, A_v_cache, A_wq, A_wo, B_x, B_w_gate, B_w_up, B_w_down, c, w_mod):

    def _A_ref(x, k_cache, v_cache, wq, wo):
        B, Sq, D = x.shape
        Hq, Dh = (32, 128)
        Hkv, Sk = (k_cache.shape[1], k_cache.shape[2])
        W = min(4096, max(256, Sk // 4))
        rep = Hq // Hkv
        q = (lambda x, *d: x.transpose(*d))((x @ wq).reshape(B, Sq, Hq, Dh), 0, 2, 1, 3)
        k = jnp.repeat(k_cache[:, :, Sk - W:, :], rep, axis=1)
        v = jnp.repeat(v_cache[:, :, Sk - W:, :], rep, axis=1)
        scores = jnp.einsum('bhqd,bhkd->bhqk', q, k) * Dh ** (-0.5)
        p = _softmax(scores, axis=-1)
        o = jnp.einsum('bhqk,bhkd->bhqd', p, v)
        return (lambda x, *d: x.transpose(*d))(o, 0, 2, 1, 3).reshape(B, Sq, Hq * Dh) @ wo

    def _B_ref(x, w_gate, w_up, w_down):
        g = jnp.einsum('bsd,df->bsf', x, w_gate)
        u = jnp.einsum('bsd,df->bsf', x, w_up)
        h = _sigmoid(g) * u
        return jnp.einsum('bsf,fd->bsd', h, w_down)
    x = A_x
    mod = (_silu(c) @ w_mod).reshape(c.shape[0], 6, 1, -1)
    sa, ca, ga, sb, cb, gb = (mod[:, 0].copy(), mod[:, 1].copy(), mod[:, 2].copy(), mod[:, 3].copy(), mod[:, 4].copy(), mod[:, 5].copy())
    h = _layernorm(x, axis=-1) * (1 + ca) + sa
    x = x + ga * _A_ref(h, A_k_cache, A_v_cache, A_wq, A_wo)
    h = _layernorm(x, axis=-1) * (1 + cb) + sb
    x = x + gb * _B_ref(h, B_w_gate, B_w_up, B_w_down)
    return x
```

```python
import functools

import jax
import jax.numpy as jnp
import jax.experimental.pallas as pl
import jax.experimental.pallas.tpu as pltpu

B = 8
D = 512
H = 32
DH = 128
SK = 4096
W = min(4096, max(256, SK // 4))
F = 1376
EPS = 1e-05
NT = (((1,), (1,)), ((), ()))
BF = jnp.bfloat16
F32 = jnp.float32


def _layernorm(x):
    m = jnp.mean(x, axis=-1, keepdims=True)
    xc = x - m
    v = jnp.mean(xc * xc, axis=-1, keepdims=True)
    return xc / jnp.sqrt(v + EPS)


def _attend(q, k_ref, v_ref):
    row = jax.lax.broadcasted_iota(jnp.int32, (B, W), 0)
    s = jnp.zeros((B, W), F32)
    for b in range(B):
        sb = jax.lax.dot_general(q, k_ref[b], NT, preferred_element_type=F32)
        s = jnp.where(row == b, sb, s)
    m = jnp.max(s, axis=-1, keepdims=True)
    p = jnp.exp(s - m)
    l = jnp.sum(p, axis=-1, keepdims=True)
    pb = p.astype(BF)
    row2 = jax.lax.broadcasted_iota(jnp.int32, (B, DH), 0)
    o = jnp.zeros((B, DH), F32)
    for b in range(B):
        ob = jnp.dot(pb, v_ref[b], preferred_element_type=F32)
        o = jnp.where(row2 == b, ob, o)
    return o / l


def _kernel(x_hbm, c_hbm, wmod_hbm, wq_hbm, k_hbm, v_hbm, wo_hbm, wg_hbm, wu_hbm, wd_hbm,
            out_ref,
            x_v, c_v, wmod_v, wq_v, wo_v, wg_v, wu_v, wd_v, kbuf, vbuf, q_s, o_s,
            wsem, ksem, vsem, *, nbuf):
    def kcp(i, slot):
        return pltpu.make_async_copy(k_hbm.at[:, i, pl.ds(SK - W, W), :], kbuf.at[slot], ksem.at[slot])

    def vcp(i, slot):
        return pltpu.make_async_copy(v_hbm.at[:, i, pl.ds(SK - W, W), :], vbuf.at[slot], vsem.at[slot])

    wcp = {}
    for j, (name, src, dst) in enumerate([
            ('c', c_hbm, c_v), ('x', x_hbm, x_v), ('wmod', wmod_hbm, wmod_v), ('wq', wq_hbm, wq_v),
            ('wo', wo_hbm, wo_v), ('wg', wg_hbm, wg_v), ('wu', wu_hbm, wu_v), ('wd', wd_hbm, wd_v)]):
        wcp[name] = pltpu.make_async_copy(src, dst, wsem.at[j])

    wcp['c'].start()
    wcp['x'].start()
    wcp['wmod'].start()
    wcp['wq'].start()
    for s in range(nbuf):
        kcp(s, s).start()
        vcp(s, s).start()

    wcp['c'].wait()
    wcp['wmod'].wait()
    c = c_v[...].astype(F32)
    sc = (c * jax.nn.sigmoid(c)).astype(BF)
    mod = jnp.dot(sc, wmod_v[...], preferred_element_type=F32)
    sa, ca, ga, sb, cb, gb = [mod[:, i * D:(i + 1) * D] for i in range(6)]
    wcp['x'].wait()
    x = x_v[...].astype(F32)
    h = (_layernorm(x) * (1.0 + ca) + sa).astype(BF)
    wcp['wq'].wait()
    q = jnp.dot(h, wq_v[...], preferred_element_type=F32) * (DH ** -0.5)
    qb = q.astype(BF)
    for i in range(H):
        q_s[i] = qb[:, i * DH:(i + 1) * DH]

    def body(i, carry):
        slot = i % nbuf
        kcp(i, slot).wait()
        vcp(i, slot).wait()
        o = _attend(q_s[i], kbuf.at[slot], vbuf.at[slot])
        o_s[i] = o.astype(BF)

        @pl.when(i + nbuf < H)
        def _():
            kcp(i + nbuf, slot).start()
            vcp(i + nbuf, slot).start()

        @pl.when(i + nbuf == H)
        def _():
            wcp['wo'].start()

        @pl.when(i + nbuf == H + 1)
        def _():
            wcp['wg'].start()
            wcp['wu'].start()
            wcp['wd'].start()
        return carry

    jax.lax.fori_loop(0, H, body, 0)

    wcp['wo'].wait()
    acc = jnp.zeros((B, D), F32)
    for i in range(H):
        acc = acc + jnp.dot(o_s[i], wo_v[pl.ds(i * DH, DH), :], preferred_element_type=F32)
    x1 = x + ga * acc
    h2 = (_layernorm(x1) * (1.0 + cb) + sb).astype(BF)
    wcp['wg'].wait()
    g = jax.lax.dot_general(h2, wg_v[...], NT, preferred_element_type=F32)
    wcp['wu'].wait()
    u = jax.lax.dot_general(h2, wu_v[...], NT, preferred_element_type=F32)
    hm = (jax.nn.sigmoid(g) * u).astype(BF)
    wcp['wd'].wait()
    y = jnp.dot(hm, wd_v[...], preferred_element_type=F32)
    out = x1 + gb * y
    out_ref[...] = out.astype(BF)


@jax.jit
def pallas_adaLN_cond__sliding_block_cached__glu_gated_glu__decode_kernel(
    A_x, A_k_cache, A_v_cache, A_wq, A_wo, B_x, B_w_gate, B_w_up, B_w_down, c, w_mod
):
    del B_x
    nbuf = 2
    hbm = pl.BlockSpec(memory_space=pltpu.HBM)
    out = pl.pallas_call(
        functools.partial(_kernel, nbuf=nbuf),
        out_shape=jax.ShapeDtypeStruct((B, D), BF),
        in_specs=[hbm] * 10,
        out_specs=pl.BlockSpec(memory_space=pltpu.VMEM),
        scratch_shapes=[
            pltpu.VMEM((B, D), BF),
            pltpu.VMEM((B, D), BF),
            pltpu.VMEM((D, 6 * D), BF),
            pltpu.VMEM((D, H * DH), BF),
            pltpu.VMEM((H * DH, D), BF),
            pltpu.VMEM((F, D), BF),
            pltpu.VMEM((F, D), BF),
            pltpu.VMEM((F, D), BF),
            pltpu.VMEM((nbuf, B, W, DH), BF),
            pltpu.VMEM((nbuf, B, W, DH), BF),
            pltpu.VMEM((H, B, DH), BF),
            pltpu.VMEM((H, B, DH), BF),
            pltpu.SemaphoreType.DMA((8,)),
            pltpu.SemaphoreType.DMA((nbuf,)),
            pltpu.SemaphoreType.DMA((nbuf,)),
        ],
        compiler_params=pltpu.CompilerParams(vmem_limit_bytes=100 * 1024 * 1024),
    )(A_x.reshape(B, D), c, w_mod, A_wq, A_k_cache, A_v_cache, A_wo,
      B_w_gate.T, B_w_up.T, B_w_down)
    return out.reshape(B, 1, D)
```

```python
import functools

import jax
import jax.numpy as jnp
import jax.experimental.pallas as pl
import jax.experimental.pallas.tpu as pltpu

B = 8
D = 512
H = 32
DH = 128
SK = 4096
W = min(4096, max(256, SK // 4))
F = 1376
EPS = 1e-05
NT = (((1,), (1,)), ((), ()))
BF = jnp.bfloat16
F32 = jnp.float32


def _layernorm(x):
    m = jnp.mean(x, axis=-1, keepdims=True)
    xc = x - m
    v = jnp.mean(xc * xc, axis=-1, keepdims=True)
    return xc / jnp.sqrt(v + EPS)


def _kernel(x_hbm, c_hbm, wmod_hbm, wq_hbm, k_hbm, v_hbm, wo_hbm, wg_hbm, wu_hbm, wd_hbm,
            out_ref,
            x_v, c_v, wmod_v, wq_v, wo_v, wg_v, wu_v, wd_v, kbuf, vbuf, q_s, o_s, hm_s,
            sem, *, pat, kvrows):
    def mo(v, m):
        return v if isinstance(v, int) else pl.multiple_of(v, m)

    def start_rows(src, dst, row0, nrows, prow, s):
        for p in range(nrows // prow):
            r = mo(row0 + p * prow, prow)
            pltpu.make_async_copy(src.at[pl.ds(r, prow), :], dst.at[pl.ds(r, prow), :], sem.at[s]).start(
                priority=pat[p % len(pat)])

    def wait_buf(buf, s):
        pltpu.make_async_copy(buf, buf, sem.at[s]).wait()

    def start_wmod(j, s):
        start_rows(wmod_hbm, wmod_v, j * 64, 64, 8, s)

    def wait_wmod(j, s):
        wait_buf(wmod_v.at[pl.ds(mo(j * 64, 64), 64), :], s)

    def start_wq(j, s):
        for p in range(8):
            r = mo(j * 32 + (p // 2) * 8, 8)
            cs = pl.ds((p % 2) * 2048, 2048)
            pltpu.make_async_copy(wq_hbm.at[pl.ds(r, 8), cs], wq_v.at[pl.ds(r, 8), cs], sem.at[s]).start(
                priority=pat[p % len(pat)])

    def wait_wq(j, s):
        wait_buf(wq_v.at[pl.ds(mo(j * 32, 32), 32), :], s)

    def start_kv(src, buf, h, b, s):
        off = 0
        for p, rows in enumerate(kvrows):
            pltpu.make_async_copy(src.at[b, h, pl.ds(SK - W + off, rows), :], buf.at[b, pl.ds(off, rows), :],
                                  sem.at[s]).start(priority=pat[p % len(pat)])
            off += rows

    cp_c = pltpu.make_async_copy(c_hbm, c_v, sem.at[8])
    cp_x = pltpu.make_async_copy(x_hbm, x_v, sem.at[8])

    cp_c.start()

    def p0(j, carry):
        start_wmod(j, 8 + j)
        return carry

    jax.lax.fori_loop(0, 8, p0, 0)
    cp_x.start()

    def p1(j, carry):
        start_wq(j, j)
        return carry

    jax.lax.fori_loop(0, 8, p1, 0)
    cp_c.wait()
    cp_x.wait()

    def p2(j, carry):
        wait_wmod(j, 8 + j)
        start_wq(8 + j, 8 + j)
        return carry

    jax.lax.fori_loop(0, 8, p2, 0)

    c = c_v[...].astype(F32)
    sc = (c * jax.nn.sigmoid(c)).astype(BF)
    mod = jnp.dot(sc, wmod_v[...], preferred_element_type=F32)
    sa, ca, ga, sb, cb, gb = [mod[:, i * D:(i + 1) * D] for i in range(6)]
    x = x_v[...].astype(F32)
    h = (_layernorm(x) * (1.0 + ca) + sa).astype(BF)

    def p3(j, carry):
        wait_wq(j, j)
        start_kv(k_hbm, kbuf, 0, j, j)
        return carry

    jax.lax.fori_loop(0, 8, p3, 0)

    def p4(j, carry):
        wait_wq(8 + j, 8 + j)
        start_kv(v_hbm, vbuf, 0, j, 8 + j)
        return carry

    jax.lax.fori_loop(0, 8, p4, 0)

    q = jnp.dot(h, wq_v[...], preferred_element_type=F32) * (DH ** -0.5)
    qb = q.astype(BF)
    for i in range(H):
        q_s[i] = qb[:, i * DH:(i + 1) * DH]

    def head(i, last):
        qh = q_s[i]
        row = jax.lax.broadcasted_iota(jnp.int32, (B, W), 0)
        s = jnp.zeros((B, W), F32)
        for b in range(B):
            wait_buf(kbuf.at[b], b)
            sb_ = jax.lax.dot_general(qh, kbuf[b], NT, preferred_element_type=F32)
            s = jnp.where(row == b, sb_, s)
            if last:
                start_rows(wo_hbm, wo_v, b * 256, 256, 32, b)
            else:
                start_kv(k_hbm, kbuf, i + 1, b, b)
        m = jnp.max(s, axis=-1, keepdims=True)
        p = jnp.exp(s - m)
        l = jnp.sum(p, axis=-1, keepdims=True)
        pb = p.astype(BF)
        row2 = jax.lax.broadcasted_iota(jnp.int32, (B, DH), 0)
        o = jnp.zeros((B, DH), F32)
        for b in range(B):
            wait_buf(vbuf.at[b], 8 + b)
            ob = jnp.dot(pb, vbuf[b], preferred_element_type=F32)
            o = jnp.where(row2 == b, ob, o)
            if last:
                start_rows(wo_hbm, wo_v, (8 + b) * 256, 256, 32, 8 + b)
            else:
                start_kv(v_hbm, vbuf, i + 1, b, 8 + b)
        o_s[i] = (o / l).astype(BF)

    def body(i, carry):
        head(i, False)
        return carry

    jax.lax.fori_loop(0, H - 1, body, 0)
    head(H - 1, True)

    def wait_wo(j):
        wait_buf(wo_v.at[pl.ds(mo(j * 256, 256), 256), :], j)

    def pace(src, dst, j0, n):
        def f(t, carry):
            wait_wo(j0 + t)
            start_rows(src, dst, t * 256, 256, 32, j0 + t)
            return carry
        jax.lax.fori_loop(0, n, f, 0)

    RL = F - 1024
    pace(wg_hbm, wg_v, 0, 4)
    wait_wo(4)
    start_rows(wg_hbm, wg_v, 1024, RL, 32, 4)
    pace(wu_hbm, wu_v, 5, 4)
    wait_wo(9)
    start_rows(wu_hbm, wu_v, 1024, RL, 32, 9)
    pace(wd_hbm, wd_v, 10, 5)
    wait_wo(15)
    start_rows(wd_hbm, wd_v, 1280, F - 1280, 32, 15)

    og = 4

    def obody(g, acc):
        for t in range(og):
            i = g * og + t
            acc = acc + jnp.dot(o_s[i], wo_v[pl.ds(pl.multiple_of(i * DH, DH), DH), :],
                                preferred_element_type=F32)
        return acc

    acc = jax.lax.fori_loop(0, H // og, obody, jnp.zeros((B, D), F32))
    x1 = x + ga * acc
    h2 = (_layernorm(x1) * (1.0 + cb) + sb).astype(BF)

    def wait_rows(buf, r0, n, s):
        wait_buf(buf.at[pl.ds(r0, n), :], s)

    for t in range(4):
        wait_rows(wg_v, t * 256, 256, t)
    wait_rows(wg_v, 1024, RL, 4)
    g = jax.lax.dot_general(h2, wg_v[...], NT, preferred_element_type=F32)
    for t in range(4):
        wait_rows(wu_v, t * 256, 256, 5 + t)
    wait_rows(wu_v, 1024, RL, 9)
    u = jax.lax.dot_general(h2, wu_v[...], NT, preferred_element_type=F32)
    hm = (jax.nn.sigmoid(g) * u).astype(BF)
    for j in range(5):
        hm_s[j] = hm[:, j * 256:(j + 1) * 256]
    hm_last = hm[:, 1280:]

    def dbody(j, y):
        rows = pl.ds(pl.multiple_of(j * 256, 256), 256)
        wait_buf(wd_v.at[rows, :], 10 + j)
        return y + jnp.dot(hm_s[j], wd_v[rows, :], preferred_element_type=F32)

    y = jax.lax.fori_loop(0, 5, dbody, jnp.zeros((B, D), F32))
    wait_rows(wd_v, 1280, F - 1280, 15)
    y = y + jnp.dot(hm_last, wd_v[pl.ds(1280, F - 1280), :], preferred_element_type=F32)
    out = x1 + gb * y
    out_ref[...] = out.astype(BF)


@jax.jit
def pallas_adaLN_cond__sliding_block_cached__glu_gated_glu__decode_kernel(
    A_x, A_k_cache, A_v_cache, A_wq, A_wo, B_x, B_w_gate, B_w_up, B_w_down, c, w_mod
):
    del B_x
    hbm = pl.BlockSpec(memory_space=pltpu.HBM)
    out = pl.pallas_call(
        functools.partial(_kernel, pat=(1, 1, 1, 0), kvrows=(128,) * 8),
        out_shape=jax.ShapeDtypeStruct((B, D), BF),
        in_specs=[hbm] * 10,
        out_specs=pl.BlockSpec(memory_space=pltpu.VMEM),
        scratch_shapes=[
            pltpu.VMEM((B, D), BF),
            pltpu.VMEM((B, D), BF),
            pltpu.VMEM((D, 6 * D), BF),
            pltpu.VMEM((D, H * DH), BF),
            pltpu.VMEM((H * DH, D), BF),
            pltpu.VMEM((F, D), BF),
            pltpu.VMEM((F, D), BF),
            pltpu.VMEM((F, D), BF),
            pltpu.VMEM((B, W, DH), BF),
            pltpu.VMEM((B, W, DH), BF),
            pltpu.VMEM((H, B, DH), BF),
            pltpu.VMEM((H, B, DH), BF),
            pltpu.VMEM((5, B, 256), BF),
            pltpu.SemaphoreType.DMA((16,)),
        ],
        compiler_params=pltpu.CompilerParams(vmem_limit_bytes=64 * 1024 * 1024),
    )(A_x.reshape(B, D), c, w_mod, A_wq, A_k_cache, A_v_cache, A_wo, B_w_gate.T, B_w_up.T, B_w_down)
    return out.reshape(B, 1, D)
```

```python
import functools

import jax
import jax.numpy as jnp
import jax.experimental.pallas as pl
import jax.experimental.pallas.tpu as pltpu

B = 8
D = 512
H = 32
DH = 128
SK = 4096
W = min(4096, max(256, SK // 4))
F = 1376
EPS = 1e-05
NT = (((1,), (1,)), ((), ()))
BF = jnp.bfloat16
F32 = jnp.float32


def _layernorm(x):
    m = jnp.mean(x, axis=-1, keepdims=True)
    xc = x - m
    v = jnp.mean(xc * xc, axis=-1, keepdims=True)
    return xc / jnp.sqrt(v + EPS)


def _kernel(x_hbm, c_hbm, wmod_hbm, wq_hbm, k_hbm, v_hbm, wo_hbm, wg_hbm, wu_hbm, wd_hbm,
            out_ref,
            x_v, c_v, wmod_v, wq_v, wo_v, wg_v, wu_v, wd_v, kbuf, vbuf, q_s, o_s,
            sem, *, order, prio, wpat, pre):
    def mo(v, m):
        return v if isinstance(v, int) else pl.multiple_of(v, m)

    def row_piece(src, dst, r, n, s, pr):
        pltpu.make_async_copy(src.at[pl.ds(r, n), :], dst.at[pl.ds(r, n), :], sem.at[s]).start(priority=pr)

    def start_rows(src, dst, row0, nrows, prow, s):
        for p in range(nrows // prow):
            row_piece(src, dst, mo(row0 + p * prow, prow), prow, s, wpat[p % len(wpat)])

    def wait_buf(buf, s):
        pltpu.make_async_copy(buf, buf, sem.at[s]).wait()

    def start_wq(j, s):
        for p in range(16):
            r = mo(j * 64 + (p // 2) * 8, 8)
            cs = pl.ds((p % 2) * 2048, 2048)
            pltpu.make_async_copy(wq_hbm.at[pl.ds(r, 8), cs], wq_v.at[pl.ds(r, 8), cs], sem.at[s]).start(
                priority=wpat[p % len(wpat)])

    PR = 2 * W // len(order)
    NPC = len(order) // 2

    def start_unit(i, b, has_k=True, has_v=True, fill=None):
        for pid, pr in zip(order, prio):
            is_k = pid < NPC
            n = pid % NPC
            if is_k and has_k:
                pltpu.make_async_copy(k_hbm.at[b, i, pl.ds(SK - W + n * PR, PR), :],
                                      kbuf.at[b, pl.ds(n * PR, PR), :], sem.at[b]).start(priority=pr)
            elif (not is_k) and has_v:
                pltpu.make_async_copy(v_hbm.at[b, i - 1, pl.ds(SK - W + n * PR, PR), :],
                                      vbuf.at[b, pl.ds(n * PR, PR), :], sem.at[b]).start(priority=pr)
            elif fill is not None:
                fill(n, pr)

    cp_c = pltpu.make_async_copy(c_hbm, c_v, sem.at[0])
    cp_x = pltpu.make_async_copy(x_hbm, x_v, sem.at[0])

    cp_c.start()
    cp_x.start()

    def p0(j, carry):
        start_rows(wmod_hbm, wmod_v, j * 64, 64, 8, j)
        return carry

    jax.lax.fori_loop(0, 8, p0, 0)
    cp_c.wait()
    cp_x.wait()

    def p1(j, carry):
        wait_buf(wmod_v.at[pl.ds(mo(j * 64, 64), 64), :], j)
        start_wq(j, j)
        return carry

    jax.lax.fori_loop(0, 8, p1, 0)

    c = c_v[...].astype(F32)
    sc = (c * jax.nn.sigmoid(c)).astype(BF)
    mod = jnp.dot(sc, wmod_v[...], preferred_element_type=F32)
    sa, ca, ga, sb, cb, gb = [mod[:, i * D:(i + 1) * D] for i in range(6)]
    x = x_v[...].astype(F32)
    h = (_layernorm(x) * (1.0 + ca) + sa).astype(BF)

    def p2(j, carry):
        wait_buf(wq_v.at[pl.ds(mo(j * 64, 64), 64), :], j)
        start_unit(0, j, has_v=False)
        return carry

    jax.lax.fori_loop(0, 8, p2, 0)

    q = jnp.dot(h, wq_v[...], preferred_element_type=F32) * (DH ** -0.5)
    qb = q.astype(BF)
    for i in range(H):
        q_s[i] = qb[:, i * DH:(i + 1) * DH]

    row = jax.lax.broadcasted_iota(jnp.int32, (B, W), 0)
    row2 = jax.lax.broadcasted_iota(jnp.int32, (B, DH), 0)

    def sweep(i, pb, linv, do_qk, do_pv, refill, wait):
        s = jnp.zeros((B, W), F32)
        o = jnp.zeros((B, DH), F32)
        qh = q_s[i] if do_qk else None
        for b in range(B):
            wait(b)
            if do_qk:
                sb_ = jax.lax.dot_general(qh, kbuf[b], NT, preferred_element_type=F32)
                s = jnp.where(row == b, sb_, s)
            if do_pv:
                ob = jnp.dot(pb, vbuf[b], preferred_element_type=F32)
                o = jnp.where(row2 == b, ob, o)
            refill(b)
        if do_pv:
            o_s[i - 1] = (o * linv).astype(BF)
        if do_qk:
            m = jnp.max(s, axis=-1, keepdims=True)
            p = jnp.exp(s - m)
            l = jnp.sum(p, axis=-1, keepdims=True)
            return p.astype(BF), 1.0 / l
        return None

    def wait_unit(b):
        wait_buf(kbuf.at[b], b)
        wait_buf(vbuf.at[b], b)

    st = sweep(0, None, None, True, False, lambda b: start_unit(1, b), lambda b: wait_buf(kbuf.at[b], b))

    def body(i, st):
        return sweep(i, st[0], st[1], True, True, lambda b: start_unit(i + 1, b), wait_unit)

    st = jax.lax.fori_loop(1, H - 1, body, st)

    def wo_fill(b):
        return lambda n, pr: row_piece(wo_hbm, wo_v, b * 256 + n * 32, 32, b, pr)

    st = sweep(H - 1, st[0], st[1], True, True,
               lambda b: start_unit(H, b, has_k=False, fill=wo_fill(b)), wait_unit)

    plan = [(wo_hbm, wo_v, 2048, 704), (wo_hbm, wo_v, 2752, 672), (wo_hbm, wo_v, 3424, 672),
            (wg_hbm, wg_v, 0, 704), (wg_hbm, wg_v, 704, 672), (wu_hbm, wu_v, 0, F),
            (wd_hbm, wd_v, 0, 1024), (wd_hbm, wd_v, 1024, F - 1024)]

    def tail_issue(b):
        src, dst, r0, n = plan[b]
        start_rows(src, dst, r0, n, 32, b)

    def tail_wait(b):
        src, dst, r0, n = plan[b]
        wait_buf(dst.at[pl.ds(r0, n), :], b)

    def wait_last_unit(b):
        wait_buf(vbuf.at[b], b)
        wait_buf(wo_v.at[pl.ds(b * 256, 256), :], b)

    sweep(H, st[0], st[1], False, True, tail_issue, wait_last_unit)

    og = 4
    for b in range(3):
        tail_wait(b)

    def obody(g, acc):
        for t in range(og):
            i = g * og + t
            acc = acc + jnp.dot(o_s[i], wo_v[pl.ds(pl.multiple_of(i * DH, DH), DH), :],
                                preferred_element_type=F32)
        return acc

    acc = jax.lax.fori_loop(0, H // og, obody, jnp.zeros((B, D), F32))
    x1 = x + ga * acc
    h2 = (_layernorm(x1) * (1.0 + cb) + sb).astype(BF)

    tail_wait(3)
    tail_wait(4)
    g = jax.lax.dot_general(h2, wg_v[...], NT, preferred_element_type=F32)
    tail_wait(5)
    u = jax.lax.dot_general(h2, wu_v[...], NT, preferred_element_type=F32)
    hm = (jax.nn.sigmoid(g) * u).astype(BF)
    for j in range(2):
        o_s[j] = hm[:, j * 512:j * 512 + 128]
        o_s[j + 2] = hm[:, j * 512 + 128:j * 512 + 256]
        o_s[j + 4] = hm[:, j * 512 + 256:j * 512 + 384]
        o_s[j + 6] = hm[:, j * 512 + 384:j * 512 + 512]
    hm_last = hm[:, 1024:]

    def dbody(j, y):
        @pl.when(j == 0)
        def _():
            tail_wait(6)
        for t in range(4):
            rows = pl.ds(pl.multiple_of(j * 512 + t * 128, 128), 128)
            y = y + jnp.dot(o_s[j + 2 * t], wd_v[rows, :], preferred_element_type=F32)
        return y

    y = jax.lax.fori_loop(0, 2, dbody, jnp.zeros((B, D), F32))
    tail_wait(7)
    y = y + jnp.dot(hm_last, wd_v[pl.ds(1024, F - 1024), :], preferred_element_type=F32)
    out = x1 + gb * y
    out_ref[...] = out.astype(BF)


@jax.jit
def pallas_adaLN_cond__sliding_block_cached__glu_gated_glu__decode_kernel(
    A_x, A_k_cache, A_v_cache, A_wq, A_wo, B_x, B_w_gate, B_w_up, B_w_down, c, w_mod
):
    del B_x
    hbm = pl.BlockSpec(memory_space=pltpu.HBM)
    out = pl.pallas_call(
        functools.partial(_kernel, order=(0, 14, 1, 15, 2, 3, 8, 9, 4, 10, 5, 11, 6, 12, 7, 13), prio=(0, 1, 1, 0, 1, 0, 0, 1, 0, 1, 1, 0, 1, 0, 0, 1), wpat=(1, 1, 1, 0), pre=0),
        out_shape=jax.ShapeDtypeStruct((B, D), BF),
        in_specs=[hbm] * 10,
        out_specs=pl.BlockSpec(memory_space=pltpu.VMEM),
        scratch_shapes=[
            pltpu.VMEM((B, D), BF),
            pltpu.VMEM((B, D), BF),
            pltpu.VMEM((D, 6 * D), BF),
            pltpu.VMEM((D, H * DH), BF),
            pltpu.VMEM((H * DH, D), BF),
            pltpu.VMEM((F, D), BF),
            pltpu.VMEM((F, D), BF),
            pltpu.VMEM((F, D), BF),
            pltpu.VMEM((B, W, DH), BF),
            pltpu.VMEM((B, W, DH), BF),
            pltpu.VMEM((H, B, DH), BF),
            pltpu.VMEM((H, B, DH), BF),
            pltpu.SemaphoreType.DMA((8,)),
        ],
        compiler_params=pltpu.CompilerParams(vmem_limit_bytes=64 * 1024 * 1024),
    )(A_x.reshape(B, D), c, w_mod, A_wq, A_k_cache, A_v_cache, A_wo, B_w_gate.T, B_w_up.T, B_w_down)
    return out.reshape(B, 1, D)
```

```python
import functools

import jax
import jax.numpy as jnp
import jax.experimental.pallas as pl
import jax.experimental.pallas.tpu as pltpu

B = 8
D = 512
H = 32
DH = 128
SK = 4096
W = min(4096, max(256, SK // 4))
F = 1376
EPS = 1e-05
NT = (((1,), (1,)), ((), ()))
BF = jnp.bfloat16
F32 = jnp.float32


def _layernorm(x):
    m = jnp.mean(x, axis=-1, keepdims=True)
    xc = x - m
    v = jnp.mean(xc * xc, axis=-1, keepdims=True)
    return xc / jnp.sqrt(v + EPS)


def _kernel(x_hbm, c_hbm, wmod_hbm, wq_hbm, k_hbm, v_hbm, wo_hbm, wg_hbm, wu_hbm, wd_hbm,
            out_ref,
            x_v, c_v, wmod_v, wq_v, wo_v, wg_v, wu_v, wd_v, kbuf, vbuf, q_s, o_s,
            sem, *, pieces, G, wpat):
    def mo(v, m):
        return v if isinstance(v, int) else pl.multiple_of(v, m)

    def row_piece(src, dst, r, n, s, pr):
        pltpu.make_async_copy(src.at[pl.ds(r, n), :], dst.at[pl.ds(r, n), :], sem.at[s]).start(priority=pr)

    def start_rows(src, dst, row0, nrows, prow, s):
        for p in range(nrows // prow):
            row_piece(src, dst, mo(row0 + p * prow, prow), prow, s, wpat[p % len(wpat)])

    def wait_buf(buf, s):
        pltpu.make_async_copy(buf, buf, sem.at[s]).wait()

    def start_wq(j, s):
        for p in range(16):
            r = mo(j * 64 + (p // 2) * 8, 8)
            cs = pl.ds((p % 2) * 2048, 2048)
            pltpu.make_async_copy(wq_hbm.at[pl.ds(r, 8), cs], wq_v.at[pl.ds(r, 8), cs], sem.at[s]).start(
                priority=wpat[p % len(wpat)])

    def start_unit(i, g, has_k=True, has_v=True, fill=None):
        for db, is_v, off, n, pr in pieces:
            b = g * G + db
            if not is_v and has_k:
                pltpu.make_async_copy(k_hbm.at[b, i, pl.ds(SK - W + off, n), :],
                                      kbuf.at[b, pl.ds(off, n), :], sem.at[g * G]).start(priority=pr)
            elif is_v and has_v:
                pltpu.make_async_copy(v_hbm.at[b, i - 1, pl.ds(SK - W + off, n), :],
                                      vbuf.at[b, pl.ds(off, n), :], sem.at[g * G]).start(priority=pr)
            elif fill is not None:
                fill(b, off, n, g * G, pr)

    cp_c = pltpu.make_async_copy(c_hbm, c_v, sem.at[0])
    cp_x = pltpu.make_async_copy(x_hbm, x_v, sem.at[0])

    cp_c.start()
    cp_x.start()

    def p0(j, carry):
        start_rows(wmod_hbm, wmod_v, j * 64, 64, 8, j)
        return carry

    jax.lax.fori_loop(0, 8, p0, 0)
    cp_c.wait()
    cp_x.wait()

    def p1(j, carry):
        wait_buf(wmod_v.at[pl.ds(mo(j * 64, 64), 64), :], j)
        start_wq(j, j)
        return carry

    jax.lax.fori_loop(0, 8, p1, 0)

    c = c_v[...].astype(F32)
    sc = (c * jax.nn.sigmoid(c)).astype(BF)
    mod = jnp.dot(sc, wmod_v[...], preferred_element_type=F32)
    sa, ca, ga, sb, cb, gb = [mod[:, i * D:(i + 1) * D] for i in range(6)]
    x = x_v[...].astype(F32)
    h = (_layernorm(x) * (1.0 + ca) + sa).astype(BF)

    def p2(g, carry):
        for db in range(G):
            j = g * G + db
            wait_buf(wq_v.at[pl.ds(mo(j * 64, 64), 64), :], j)
        start_unit(0, g, has_v=False)
        return carry

    jax.lax.fori_loop(0, B // G, p2, 0)

    q = jnp.dot(h, wq_v[...], preferred_element_type=F32) * (DH ** -0.5)
    qb = q.astype(BF)
    for i in range(H):
        q_s[i] = qb[:, i * DH:(i + 1) * DH]

    row = jax.lax.broadcasted_iota(jnp.int32, (B, W), 0)
    row2 = jax.lax.broadcasted_iota(jnp.int32, (B, DH), 0)

    def sweep(i, pb, linv, do_qk, do_pv, refill, wait):
        s = jnp.zeros((B, W), F32)
        o = jnp.zeros((B, DH), F32)
        qh = q_s[i] if do_qk else None
        for b in range(B):
            if b % G == 0:
                wait(b)
            if do_qk:
                sb_ = jax.lax.dot_general(qh, kbuf[b], NT, preferred_element_type=F32)
                s = jnp.where(row == b, sb_, s)
            if do_pv:
                ob = jnp.dot(pb, vbuf[b], preferred_element_type=F32)
                o = jnp.where(row2 == b, ob, o)
            if b % G == G - 1:
                refill(b // G)
        if do_pv:
            o_s[i - 1] = (o * linv).astype(BF)
        if do_qk:
            m = jnp.max(s, axis=-1, keepdims=True)
            p = jnp.exp(s - m)
            l = jnp.sum(p, axis=-1, keepdims=True)
            return p.astype(BF), 1.0 / l
        return None

    def wait_k(b):
        wait_buf(kbuf.at[pl.ds(b, G)], b)

    def wait_unit(b):
        wait_buf(kbuf.at[pl.ds(b, G)], b)
        wait_buf(vbuf.at[pl.ds(b, G)], b)

    st = sweep(0, None, None, True, False, lambda g: start_unit(1, g), wait_k)

    def body(i, st):
        return sweep(i, st[0], st[1], True, True, lambda g: start_unit(i + 1, g), wait_unit)

    st = jax.lax.fori_loop(1, H - 1, body, st)

    def wo_fill(b, off, n, s, pr):
        row_piece(wo_hbm, wo_v, b * 256 + off // 4, n // 4, s, pr)

    st = sweep(H - 1, st[0], st[1], True, True,
               lambda g: start_unit(H, g, has_k=False, fill=wo_fill), wait_unit)

    plan = [(wo_hbm, wo_v, 2048, 704), (wo_hbm, wo_v, 2752, 672), (wo_hbm, wo_v, 3424, 672),
            (wg_hbm, wg_v, 0, 704), (wg_hbm, wg_v, 704, 672), (wu_hbm, wu_v, 0, F),
            (wd_hbm, wd_v, 0, 1024), (wd_hbm, wd_v, 1024, F - 1024)]

    def tail_issue(g):
        for b in range(g * G, g * G + G):
            src, dst, r0, n = plan[b]
            start_rows(src, dst, r0, n, 32, b)

    def tail_wait(b):
        src, dst, r0, n = plan[b]
        wait_buf(dst.at[pl.ds(r0, n), :], b)

    def wait_last_unit(b):
        wait_buf(vbuf.at[pl.ds(b, G)], b)
        wait_buf(wo_v.at[pl.ds(b * 256, 256 * G), :], b)

    sweep(H, st[0], st[1], False, True, tail_issue, wait_last_unit)

    og = 4
    for b in range(3):
        tail_wait(b)

    def obody(g, acc):
        for t in range(og):
            i = g * og + t
            acc = acc + jnp.dot(o_s[i], wo_v[pl.ds(pl.multiple_of(i * DH, DH), DH), :],
                                preferred_element_type=F32)
        return acc

    acc = jax.lax.fori_loop(0, H // og, obody, jnp.zeros((B, D), F32))
    x1 = x + ga * acc
    h2 = (_layernorm(x1) * (1.0 + cb) + sb).astype(BF)

    tail_wait(3)
    tail_wait(4)
    g = jax.lax.dot_general(h2, wg_v[...], NT, preferred_element_type=F32)
    tail_wait(5)
    u = jax.lax.dot_general(h2, wu_v[...], NT, preferred_element_type=F32)
    hm = (jax.nn.sigmoid(g) * u).astype(BF)
    for j in range(2):
        o_s[j] = hm[:, j * 512:j * 512 + 128]
        o_s[j + 2] = hm[:, j * 512 + 128:j * 512 + 256]
        o_s[j + 4] = hm[:, j * 512 + 256:j * 512 + 384]
        o_s[j + 6] = hm[:, j * 512 + 384:j * 512 + 512]
    hm_last = hm[:, 1024:]

    def dbody(j, y):
        @pl.when(j == 0)
        def _():
            tail_wait(6)
        for t in range(4):
            rows = pl.ds(pl.multiple_of(j * 512 + t * 128, 128), 128)
            y = y + jnp.dot(o_s[j + 2 * t], wd_v[rows, :], preferred_element_type=F32)
        return y

    y = jax.lax.fori_loop(0, 2, dbody, jnp.zeros((B, D), F32))
    tail_wait(7)
    y = y + jnp.dot(hm_last, wd_v[pl.ds(1024, F - 1024), :], preferred_element_type=F32)
    out = x1 + gb * y
    out_ref[...] = out.astype(BF)


KV_PIECES = (
    (0, 0, 0, 64, 1), (0, 0, 64, 128, 0), (0, 1, 0, 128, 1), (0, 1, 128, 128, 0),
    (1, 0, 0, 64, 1), (1, 0, 64, 128, 0), (1, 1, 0, 128, 1), (1, 1, 128, 128, 0),
    (0, 0, 192, 128, 0), (0, 0, 320, 128, 1), (0, 1, 256, 128, 0), (0, 1, 384, 128, 1),
    (1, 0, 192, 128, 0), (1, 0, 320, 128, 1), (1, 1, 256, 128, 0), (1, 1, 384, 128, 1),
    (0, 0, 448, 128, 1), (0, 0, 576, 128, 0), (0, 1, 512, 128, 1), (0, 1, 640, 128, 0),
    (1, 0, 448, 128, 1), (1, 0, 576, 128, 0), (1, 1, 512, 128, 1), (1, 1, 640, 128, 0),
    (0, 0, 704, 128, 0), (0, 0, 832, 128, 1), (0, 1, 768, 128, 0), (0, 1, 896, 128, 1),
    (1, 0, 704, 128, 0), (1, 0, 832, 128, 1), (1, 1, 768, 128, 0), (1, 1, 896, 128, 1),
    (0, 0, 960, 64, 1), (1, 0, 960, 64, 1),
)


@jax.jit
def pallas_adaLN_cond__sliding_block_cached__glu_gated_glu__decode_kernel(
    A_x, A_k_cache, A_v_cache, A_wq, A_wo, B_x, B_w_gate, B_w_up, B_w_down, c, w_mod
):
    del B_x
    hbm = pl.BlockSpec(memory_space=pltpu.HBM)
    out = pl.pallas_call(
        functools.partial(_kernel, pieces=KV_PIECES, G=2, wpat=(1, 1, 1, 0)),
        out_shape=jax.ShapeDtypeStruct((B, D), BF),
        in_specs=[hbm] * 10,
        out_specs=pl.BlockSpec(memory_space=pltpu.VMEM),
        scratch_shapes=[
            pltpu.VMEM((B, D), BF),
            pltpu.VMEM((B, D), BF),
            pltpu.VMEM((D, 6 * D), BF),
            pltpu.VMEM((D, H * DH), BF),
            pltpu.VMEM((H * DH, D), BF),
            pltpu.VMEM((F, D), BF),
            pltpu.VMEM((F, D), BF),
            pltpu.VMEM((F, D), BF),
            pltpu.VMEM((B, W, DH), BF),
            pltpu.VMEM((B, W, DH), BF),
            pltpu.VMEM((H, B, DH), BF),
            pltpu.VMEM((H, B, DH), BF),
            pltpu.SemaphoreType.DMA((8,)),
        ],
        compiler_params=pltpu.CompilerParams(vmem_limit_bytes=64 * 1024 * 1024),
    )(A_x.reshape(B, D), c, w_mod, A_wq, A_k_cache, A_v_cache, A_wo, B_w_gate.T, B_w_up.T, B_w_down)
    return out.reshape(B, 1, D)
```

```python
import functools

import jax
import jax.numpy as jnp
import jax.experimental.pallas as pl
import jax.experimental.pallas.tpu as pltpu

B = 8
D = 512
H = 32
DH = 128
SK = 4096
W = min(4096, max(256, SK // 4))
F = 1376
EPS = 1e-05
NT = (((1,), (1,)), ((), ()))
BF = jnp.bfloat16
F32 = jnp.float32


def _layernorm(x):
    m = jnp.mean(x, axis=-1, keepdims=True)
    xc = x - m
    v = jnp.mean(xc * xc, axis=-1, keepdims=True)
    return xc / jnp.sqrt(v + EPS)


def _kernel(x_hbm, c_hbm, wmod_hbm, wq_hbm, k_hbm, v_hbm, wo_hbm, wg_hbm, wu_hbm, wd_hbm,
            out_ref,
            x_v, c_v, wmod_v, wq_v, wo_v, wg_v, wu_v, wd_v, kbuf, vbuf, q_s, o_s,
            sem, *, pieces, G, wcfg):
    def mo(v, m):
        return v if isinstance(v, int) else pl.multiple_of(v, m)

    def row_piece(src, dst, r, n, s, pr):
        pltpu.make_async_copy(src.at[pl.ds(r, n), :], dst.at[pl.ds(r, n), :], sem.at[s]).start(priority=pr)

    def start_rows(src, dst, row0, nrows, s, cfg):
        delta, mode = cfg
        cols = src.shape[1]
        if cols == 512:
            halves = [(16 * j, 16, 0, 512) for j in range(nrows // 16)]
        else:
            per = cols // 1024
            halves = [(8 * (j // per), 8, 1024 * (j % per), 1024) for j in range(nrows // 8 * per)]
        blocks = {}
        for j, hb in enumerate(halves):
            blocks.setdefault((j + delta) // 2, []).append(hb)
        tm = lambda m: (m ^ (m >> 1)) & 1
        span, qs, pk = mode
        key = lambda m: (m // span, m % qs // 2, m % span // qs, m % 2)
        prio = [lambda m: tm(m), lambda m: 1 - tm(m), lambda m: m & 1, lambda m: 1 - (m & 1),
                lambda m: (m >> 1) & 1, lambda m: 1 - ((m >> 1) & 1), lambda m: int(m % 4 != 3),
                lambda m: tm(m) ^ ((m >> 2) & 1), lambda m: 1 ^ tm(m) ^ ((m >> 2) & 1)][pk]
        for m in sorted(blocks, key=key):
            hbs = blocks[m]
            if len(hbs) == 2:
                (r0, n0, c0, w0), (r1, n1, c1, w1) = hbs
                if c0 == c1:
                    hbs = [(r0, n0 + n1, c0, w0)]
                elif r0 == r1:
                    hbs = [(r0, n0, c0, w0 + w1)]
            for r, n, c, w in hbs:
                rows = pl.ds(mo(row0 + r, 8), n)
                pltpu.make_async_copy(src.at[rows, pl.ds(c, w)], dst.at[rows, pl.ds(c, w)], sem.at[s]).start(
                    priority=prio(m))

    def wait_buf(buf, s):
        pltpu.make_async_copy(buf, buf, sem.at[s]).wait()

    def start_unit(i, g, has_k=True, has_v=True, fill=None):
        for db, is_v, off, n, pr in pieces:
            b = g * G + db
            if not is_v and has_k:
                pltpu.make_async_copy(k_hbm.at[b, i, pl.ds(SK - W + off, n), :],
                                      kbuf.at[b, pl.ds(off, n), :], sem.at[g]).start(priority=pr)
            elif is_v and has_v:
                pltpu.make_async_copy(v_hbm.at[b, i - 1, pl.ds(SK - W + off, n), :],
                                      vbuf.at[b, pl.ds(off, n), :], sem.at[g]).start(priority=pr)
            elif fill is not None:
                fill(b, off, n, g, pr)

    cp_c = pltpu.make_async_copy(c_hbm, c_v, sem.at[0])
    cp_x = pltpu.make_async_copy(x_hbm, x_v, sem.at[0])

    cp_c.start()
    cp_x.start()

    NG = B // G
    RG = D // NG

    def p0(j, carry):
        start_rows(wmod_hbm, wmod_v, j * RG, RG, j, wcfg[0])
        return carry

    jax.lax.fori_loop(0, NG, p0, 0)
    cp_c.wait()
    cp_x.wait()

    def p1(j, carry):
        wait_buf(wmod_v.at[pl.ds(mo(j * RG, RG), RG), :], j)
        start_rows(wq_hbm, wq_v, j * RG, RG, j, wcfg[1])
        return carry

    jax.lax.fori_loop(0, NG, p1, 0)

    c = c_v[...].astype(F32)
    sc = (c * jax.nn.sigmoid(c)).astype(BF)
    mod = jnp.dot(sc, wmod_v[...], preferred_element_type=F32)
    sa, ca, ga, sb, cb, gb = [mod[:, i * D:(i + 1) * D] for i in range(6)]
    x = x_v[...].astype(F32)
    h = (_layernorm(x) * (1.0 + ca) + sa).astype(BF)

    def p2(g, carry):
        wait_buf(wq_v.at[pl.ds(mo(g * RG, RG), RG), :], g)
        start_unit(0, g, has_v=False)
        return carry

    jax.lax.fori_loop(0, NG, p2, 0)

    q = jnp.dot(h, wq_v[...], preferred_element_type=F32) * (DH ** -0.5)
    qb = q.astype(BF)
    for i in range(H):
        q_s[i] = qb[:, i * DH:(i + 1) * DH]

    row = jax.lax.broadcasted_iota(jnp.int32, (B, W), 0)
    row2 = jax.lax.broadcasted_iota(jnp.int32, (B, DH), 0)

    def sweep(i, pb, linv, do_qk, do_pv, refill, wait):
        s = jnp.zeros((B, W), F32)
        o = jnp.zeros((B, DH), F32)
        qh = q_s[i] if do_qk else None
        for b in range(B):
            if b % G == 0:
                wait(b)
            if do_qk:
                sb_ = jax.lax.dot_general(qh, kbuf[b], NT, preferred_element_type=F32)
                s = jnp.where(row == b, sb_, s)
            if do_pv:
                ob = jnp.dot(pb, vbuf[b], preferred_element_type=F32)
                o = jnp.where(row2 == b, ob, o)
            if b % G == G - 1:
                refill(b // G)
        if do_pv:
            o_s[i - 1] = (o * linv).astype(BF)
        if do_qk:
            m = jnp.max(s, axis=-1, keepdims=True)
            p = jnp.exp(s - m)
            l = jnp.sum(p, axis=-1, keepdims=True)
            return p.astype(BF), 1.0 / l
        return None

    def wait_k(b):
        wait_buf(kbuf.at[pl.ds(b, G)], b // G)

    def wait_unit(b):
        wait_buf(kbuf.at[pl.ds(b, G)], b // G)
        wait_buf(vbuf.at[pl.ds(b, G)], b // G)

    st = sweep(0, None, None, True, False, lambda g: start_unit(1, g), wait_k)

    def body(i, st):
        return sweep(i, st[0], st[1], True, True, lambda g: start_unit(i + 1, g), wait_unit)

    st = jax.lax.fori_loop(1, H - 1, body, st)

    def wo_fill(b, off, n, s, pr):
        if wcfg[2] is None:
            row_piece(wo_hbm, wo_v, b * 256 + off // 4, n // 4, s, pr)
        elif off == 0 and b % G == 0:
            start_rows(wo_hbm, wo_v, b * 256, 256 * G, s, wcfg[2])

    st = sweep(H - 1, st[0], st[1], True, True,
               lambda g: start_unit(H, g, has_k=False, fill=wo_fill), wait_unit)

    plan = [(wo_hbm, wo_v, 2048, 1024, 0, 3), (wo_hbm, wo_v, 3072, 1024, 1, 3), (wg_hbm, wg_v, 0, F, 2, 4),
            (wu_hbm, wu_v, 0, F, 3, 5), (wd_hbm, wd_v, 0, 1024, 0, 6), (wd_hbm, wd_v, 1024, F - 1024, 1, 6)]

    def tail_issue(t):
        src, dst, r0, n, s, w = plan[t]
        start_rows(src, dst, r0, n, s, wcfg[w])

    def tail_wait(t):
        src, dst, r0, n, s, w = plan[t]
        wait_buf(dst.at[pl.ds(r0, n), :], s)

    def wait_last_unit(b):
        wait_buf(vbuf.at[pl.ds(b, G)], b // G)
        wait_buf(wo_v.at[pl.ds(b * 256, 256 * G), :], b // G)

    sweep(H, st[0], st[1], False, True, tail_issue, wait_last_unit)

    og = 4
    tail_wait(0)
    tail_issue(4)
    tail_wait(1)
    tail_issue(5)

    def obody(g, acc):
        for t in range(og):
            i = g * og + t
            acc = acc + jnp.dot(o_s[i], wo_v[pl.ds(pl.multiple_of(i * DH, DH), DH), :],
                                preferred_element_type=F32)
        return acc

    acc = jax.lax.fori_loop(0, H // og, obody, jnp.zeros((B, D), F32))
    x1 = x + ga * acc
    h2 = (_layernorm(x1) * (1.0 + cb) + sb).astype(BF)

    tail_wait(2)
    g = jax.lax.dot_general(h2, wg_v[...], NT, preferred_element_type=F32)
    tail_wait(3)
    u = jax.lax.dot_general(h2, wu_v[...], NT, preferred_element_type=F32)
    hm = (jax.nn.sigmoid(g) * u).astype(BF)
    for j in range(2):
        o_s[j] = hm[:, j * 512:j * 512 + 128]
        o_s[j + 2] = hm[:, j * 512 + 128:j * 512 + 256]
        o_s[j + 4] = hm[:, j * 512 + 256:j * 512 + 384]
        o_s[j + 6] = hm[:, j * 512 + 384:j * 512 + 512]
    hm_last = hm[:, 1024:]

    def dbody(j, y):
        @pl.when(j == 0)
        def _():
            tail_wait(4)
        for t in range(4):
            rows = pl.ds(pl.multiple_of(j * 512 + t * 128, 128), 128)
            y = y + jnp.dot(o_s[j + 2 * t], wd_v[rows, :], preferred_element_type=F32)
        return y

    y = jax.lax.fori_loop(0, 2, dbody, jnp.zeros((B, D), F32))
    tail_wait(5)
    y = y + jnp.dot(hm_last, wd_v[pl.ds(1024, F - 1024), :], preferred_element_type=F32)
    out = x1 + gb * y
    out_ref[...] = out.astype(BF)


WEIGHT_PIECES = ((0, (32, 4, 1)), (1, (32, 4, 1)), None) + ((1, (32, 4, 1)),) * 4

KV_PIECES = (
    (0, 0, 0, 64, 0), (1, 0, 64, 128, 1), (1, 1, 896, 128, 0), (1, 0, 0, 64, 0),
    (0, 1, 0, 128, 0), (1, 1, 128, 128, 1), (0, 1, 128, 128, 1), (1, 1, 0, 128, 0),
    (0, 1, 256, 128, 1), (0, 0, 192, 128, 1), (0, 1, 384, 128, 0), (0, 0, 320, 128, 1),
    (1, 0, 192, 128, 1), (1, 0, 320, 128, 0), (1, 1, 256, 128, 1), (1, 1, 384, 128, 0),
    (0, 0, 448, 128, 1), (0, 1, 512, 128, 0), (0, 0, 576, 128, 1), (1, 0, 448, 128, 0),
    (1, 0, 576, 128, 1), (1, 1, 512, 128, 0), (0, 0, 704, 128, 1), (1, 1, 640, 128, 1),
    (0, 0, 832, 128, 0), (0, 1, 640, 128, 1), (0, 1, 768, 128, 1), (0, 1, 896, 128, 0),
    (1, 0, 704, 128, 1), (1, 0, 832, 128, 0), (1, 1, 768, 128, 1), (0, 0, 64, 128, 1),
    (0, 0, 960, 64, 0), (1, 0, 960, 64, 0),
)


@jax.jit
def pallas_adaLN_cond__sliding_block_cached__glu_gated_glu__decode_kernel(
    A_x, A_k_cache, A_v_cache, A_wq, A_wo, B_x, B_w_gate, B_w_up, B_w_down, c, w_mod
):
    del B_x
    hbm = pl.BlockSpec(memory_space=pltpu.HBM)
    out = pl.pallas_call(
        functools.partial(_kernel, pieces=KV_PIECES, G=2, wcfg=WEIGHT_PIECES),
        out_shape=jax.ShapeDtypeStruct((B, D), BF),
        in_specs=[hbm] * 10,
        out_specs=pl.BlockSpec(memory_space=pltpu.VMEM),
        scratch_shapes=[
            pltpu.VMEM((B, D), BF),
            pltpu.VMEM((B, D), BF),
            pltpu.VMEM((D, 6 * D), BF),
            pltpu.VMEM((D, H * DH), BF),
            pltpu.VMEM((H * DH, D), BF),
            pltpu.VMEM((F, D), BF),
            pltpu.VMEM((F, D), BF),
            pltpu.VMEM((F, D), BF),
            pltpu.VMEM((B, W, DH), BF),
            pltpu.VMEM((B, W, DH), BF),
            pltpu.VMEM((H, B, DH), BF),
            pltpu.VMEM((H, B, DH), BF),
            pltpu.SemaphoreType.DMA((B // G,)),
        ],
        compiler_params=pltpu.CompilerParams(vmem_limit_bytes=64 * 1024 * 1024),
    )(A_x.reshape(B, D), c, w_mod, A_wq, A_k_cache, A_v_cache, A_wo, B_w_gate.T, B_w_up.T, B_w_down)
    return out.reshape(B, 1, D)
```

```python
import functools

import jax
import jax.numpy as jnp
import jax.experimental.pallas as pl
import jax.experimental.pallas.tpu as pltpu

B = 8
D = 512
H = 32
DH = 128
SK = 4096
W = min(4096, max(256, SK // 4))
F = 1376
EPS = 1e-05
NT = (((1,), (1,)), ((), ()))
BF = jnp.bfloat16
F32 = jnp.float32


def _layernorm(x):
    m = jnp.mean(x, axis=-1, keepdims=True)
    xc = x - m
    v = jnp.mean(xc * xc, axis=-1, keepdims=True)
    return xc / jnp.sqrt(v + EPS)


def _kernel(x_hbm, c_hbm, wmod_hbm, wq_hbm, k_hbm, v_hbm, wo_hbm, wg_hbm, wu_hbm, wd_hbm,
            out_ref,
            x_v, c_v, wmod_v, wq_v, wo_v, wg_v, wu_v, wd_v, kbuf, vbuf, q_s, o_s,
            sem, *, pieces, G, wcfg):
    def mo(v, m):
        return v if isinstance(v, int) else pl.multiple_of(v, m)

    def row_piece(src, dst, r, n, s, pr):
        pltpu.make_async_copy(src.at[pl.ds(r, n), :], dst.at[pl.ds(r, n), :], sem.at[s]).start(priority=pr)

    def start_rows(src, dst, row0, nrows, s, cfg):
        delta, mode = cfg
        cols = src.shape[1]
        if cols == 512:
            halves = [(16 * j, 16, 0, 512) for j in range(nrows // 16)]
        else:
            per = cols // 1024
            halves = [(8 * (j // per), 8, 1024 * (j % per), 1024) for j in range(nrows // 8 * per)]
        blocks = {}
        for j, hb in enumerate(halves):
            blocks.setdefault((j + delta) // 2, []).append(hb)
        tm = lambda m: (m ^ (m >> 1)) & 1
        span, qs, pk = mode
        key = lambda m: (m // span, m % qs // 2, m % span // qs, m % 2)
        prio = [lambda m: tm(m), lambda m: 1 - tm(m), lambda m: m & 1, lambda m: 1 - (m & 1),
                lambda m: (m >> 1) & 1, lambda m: 1 - ((m >> 1) & 1), lambda m: int(m % 4 != 3),
                lambda m: tm(m) ^ ((m >> 2) & 1), lambda m: 1 ^ tm(m) ^ ((m >> 2) & 1)][pk]
        for m in sorted(blocks, key=key):
            hbs = blocks[m]
            if len(hbs) == 2:
                (r0, n0, c0, w0), (r1, n1, c1, w1) = hbs
                if c0 == c1:
                    hbs = [(r0, n0 + n1, c0, w0)]
                elif r0 == r1:
                    hbs = [(r0, n0, c0, w0 + w1)]
            for r, n, c, w in hbs:
                rows = pl.ds(mo(row0 + r, 8), n)
                pltpu.make_async_copy(src.at[rows, pl.ds(c, w)], dst.at[rows, pl.ds(c, w)], sem.at[s]).start(
                    priority=prio(m))

    def wait_buf(buf, s):
        pltpu.make_async_copy(buf, buf, sem.at[s]).wait()

    def start_unit(i, g, has_k=True, has_v=True, fill=None):
        for db, is_v, off, n, pr in pieces:
            b = g * G + db
            if not is_v and has_k:
                pltpu.make_async_copy(k_hbm.at[b, i, pl.ds(SK - W + off, n), :],
                                      kbuf.at[b, pl.ds(off, n), :], sem.at[g]).start(priority=pr)
            elif is_v and has_v:
                pltpu.make_async_copy(v_hbm.at[b, i - 1, pl.ds(SK - W + off, n), :],
                                      vbuf.at[b, pl.ds(off, n), :], sem.at[g]).start(priority=pr)
            elif fill is not None:
                fill(b, off, n, g, pr)

    cp_c = pltpu.make_async_copy(c_hbm, c_v, sem.at[0])
    cp_x = pltpu.make_async_copy(x_hbm, x_v, sem.at[0])

    cp_c.start()
    cp_x.start()

    NG = B // G
    RG = D // NG

    def p0(j, carry):
        start_rows(wmod_hbm, wmod_v, j * RG, RG, j, wcfg[0])
        return carry

    jax.lax.fori_loop(0, NG, p0, 0)
    cp_c.wait()
    cp_x.wait()

    def p1(j, carry):
        wait_buf(wmod_v.at[pl.ds(mo(j * RG, RG), RG), :], j)
        start_rows(wq_hbm, wq_v, j * RG, RG, j, wcfg[1])
        return carry

    jax.lax.fori_loop(0, NG, p1, 0)

    c = c_v[...].astype(F32)
    sc = (c * jax.nn.sigmoid(c)).astype(BF)
    mod = jnp.dot(sc, wmod_v[...], preferred_element_type=F32)
    sa, ca, ga, sb, cb, gb = [mod[:, i * D:(i + 1) * D] for i in range(6)]
    x = x_v[...].astype(F32)
    h = (_layernorm(x) * (1.0 + ca) + sa).astype(BF)

    def p2(g, carry):
        wait_buf(wq_v.at[pl.ds(mo(g * RG, RG), RG), :], g)
        start_unit(0, g, has_v=False)
        return carry

    jax.lax.fori_loop(0, NG, p2, 0)

    q = jnp.dot(h, wq_v[...], preferred_element_type=F32) * (DH ** -0.5)
    qb = q.astype(BF)
    for i in range(H):
        q_s[i] = qb[:, i * DH:(i + 1) * DH]

    row = jax.lax.broadcasted_iota(jnp.int32, (B, W), 0)
    row2 = jax.lax.broadcasted_iota(jnp.int32, (B, DH), 0)

    def sweep(i, pb, linv, do_qk, do_pv, refill, wait):
        s = jnp.zeros((B, W), F32)
        o = jnp.zeros((B, DH), F32)
        qh = q_s[i] if do_qk else None
        for b in range(B):
            if b % G == 0:
                wait(b)
            if do_qk:
                sb_ = jax.lax.dot_general(qh, kbuf[b], NT, preferred_element_type=F32)
                s = jnp.where(row == b, sb_, s)
            if do_pv:
                ob = jnp.dot(pb, vbuf[b], preferred_element_type=F32)
                o = jnp.where(row2 == b, ob, o)
            if b % G == G - 1:
                refill(b // G)
        if do_pv:
            o_s[i - 1] = (o * linv).astype(BF)
        if do_qk:
            m = jnp.max(s, axis=-1, keepdims=True)
            p = jnp.exp(s - m)
            l = jnp.sum(p, axis=-1, keepdims=True)
            return p.astype(BF), 1.0 / l
        return None

    def wait_k(b):
        wait_buf(kbuf.at[pl.ds(b, G)], b // G)

    def wait_unit(b):
        wait_buf(kbuf.at[pl.ds(b, G)], b // G)
        wait_buf(vbuf.at[pl.ds(b, G)], b // G)

    st = sweep(0, None, None, True, False, lambda g: start_unit(1, g), wait_k)

    def body(i, st):
        return sweep(i, st[0], st[1], True, True, lambda g: start_unit(i + 1, g), wait_unit)

    st = jax.lax.fori_loop(1, H - 1, body, st)

    def wo_fill(b, off, n, s, pr):
        if wcfg[2] is None:
            row_piece(wo_hbm, wo_v, b * 256 + off // 4, n // 4, s, pr)
        elif off == 0 and b % G == 0:
            start_rows(wo_hbm, wo_v, b * 256, 256 * G, s, wcfg[2])

    st = sweep(H - 1, st[0], st[1], True, True,
               lambda g: start_unit(H, g, has_k=False, fill=wo_fill), wait_unit)

    plan = [(wo_hbm, wo_v, 2048, 1024, 0, 3), (wo_hbm, wo_v, 3072, 1024, 1, 3), (wg_hbm, wg_v, 0, F, 2, 4),
            (wu_hbm, wu_v, 0, F, 3, 5), (wd_hbm, wd_v, 0, 1024, 0, 6), (wd_hbm, wd_v, 1024, F - 1024, 1, 6)]

    def tail_issue(t):
        src, dst, r0, n, s, w = plan[t]
        start_rows(src, dst, r0, n, s, wcfg[w])

    def tail_wait(t):
        src, dst, r0, n, s, w = plan[t]
        wait_buf(dst.at[pl.ds(r0, n), :], s)

    def wait_last_unit(b):
        wait_buf(vbuf.at[pl.ds(b, G)], b // G)
        wait_buf(wo_v.at[pl.ds(b * 256, 256 * G), :], b // G)

    sweep(H, st[0], st[1], False, True, tail_issue, wait_last_unit)

    og = 4
    tail_wait(0)
    tail_issue(4)
    tail_wait(1)
    tail_issue(5)

    def obody(g, acc):
        for t in range(og):
            i = g * og + t
            acc = acc + jnp.dot(o_s[i], wo_v[pl.ds(pl.multiple_of(i * DH, DH), DH), :],
                                preferred_element_type=F32)
        return acc

    acc = jax.lax.fori_loop(0, H // og, obody, jnp.zeros((B, D), F32))
    x1 = x + ga * acc
    h2 = (_layernorm(x1) * (1.0 + cb) + sb).astype(BF)

    tail_wait(2)
    g = jax.lax.dot_general(h2, wg_v[...], NT, preferred_element_type=F32)
    tail_wait(3)
    u = jax.lax.dot_general(h2, wu_v[...], NT, preferred_element_type=F32)
    hm = (jax.nn.sigmoid(g) * u).astype(BF)
    for j in range(2):
        o_s[j] = hm[:, j * 512:j * 512 + 128]
        o_s[j + 2] = hm[:, j * 512 + 128:j * 512 + 256]
        o_s[j + 4] = hm[:, j * 512 + 256:j * 512 + 384]
        o_s[j + 6] = hm[:, j * 512 + 384:j * 512 + 512]
    hm_last = hm[:, 1024:]

    def dbody(j, y):
        @pl.when(j == 0)
        def _():
            tail_wait(4)
        for t in range(4):
            rows = pl.ds(pl.multiple_of(j * 512 + t * 128, 128), 128)
            y = y + jnp.dot(o_s[j + 2 * t], wd_v[rows, :], preferred_element_type=F32)
        return y

    y = jax.lax.fori_loop(0, 2, dbody, jnp.zeros((B, D), F32))
    tail_wait(5)
    y = y + jnp.dot(hm_last, wd_v[pl.ds(1024, F - 1024), :], preferred_element_type=F32)
    out = x1 + gb * y
    out_ref[...] = out.astype(BF)


WEIGHT_PIECES = ((0, (32, 4, 1)), (1, (32, 4, 1)), None) + ((1, (32, 4, 1)),) * 4

KV_PIECES = (
    (0, 0, 0, 64, 0), (1, 0, 64, 128, 1), (1, 0, 0, 64, 0), (1, 1, 896, 128, 0),
    (1, 1, 128, 128, 1), (1, 1, 0, 128, 0), (0, 1, 256, 128, 1), (0, 1, 384, 128, 0),
    (0, 0, 192, 128, 1), (0, 0, 320, 128, 1), (1, 0, 192, 128, 1), (0, 1, 128, 128, 1),
    (1, 0, 320, 128, 1), (1, 1, 256, 128, 1), (1, 1, 384, 128, 0), (0, 0, 448, 128, 1),
    (0, 1, 512, 128, 0), (0, 0, 576, 128, 1), (1, 0, 448, 128, 0), (1, 0, 576, 128, 1),
    (0, 1, 768, 128, 1), (0, 1, 640, 128, 1), (0, 0, 704, 128, 1), (1, 1, 640, 128, 1),
    (1, 1, 512, 128, 0), (0, 0, 832, 128, 0), (0, 1, 0, 128, 0), (0, 1, 896, 128, 0),
    (1, 0, 704, 128, 1), (1, 0, 832, 128, 0), (1, 1, 768, 128, 1), (0, 0, 64, 128, 1),
    (0, 0, 960, 64, 0), (1, 0, 960, 64, 0),
)


@jax.jit
def pallas_adaLN_cond__sliding_block_cached__glu_gated_glu__decode_kernel(
    A_x, A_k_cache, A_v_cache, A_wq, A_wo, B_x, B_w_gate, B_w_up, B_w_down, c, w_mod
):
    del B_x
    hbm = pl.BlockSpec(memory_space=pltpu.HBM)
    out = pl.pallas_call(
        functools.partial(_kernel, pieces=KV_PIECES, G=2, wcfg=WEIGHT_PIECES),
        out_shape=jax.ShapeDtypeStruct((B, D), BF),
        in_specs=[hbm] * 10,
        out_specs=pl.BlockSpec(memory_space=pltpu.VMEM),
        scratch_shapes=[
            pltpu.VMEM((B, D), BF),
            pltpu.VMEM((B, D), BF),
            pltpu.VMEM((D, 6 * D), BF),
            pltpu.VMEM((D, H * DH), BF),
            pltpu.VMEM((H * DH, D), BF),
            pltpu.VMEM((F, D), BF),
            pltpu.VMEM((F, D), BF),
            pltpu.VMEM((F, D), BF),
            pltpu.VMEM((B, W, DH), BF),
            pltpu.VMEM((B, W, DH), BF),
            pltpu.VMEM((H, B, DH), BF),
            pltpu.VMEM((H, B, DH), BF),
            pltpu.SemaphoreType.DMA((B // 2,)),
        ],
        compiler_params=pltpu.CompilerParams(vmem_limit_bytes=64 * 1024 * 1024),
    )(A_x.reshape(B, D), c, w_mod, A_wq, A_k_cache, A_v_cache, A_wo, B_w_gate.T, B_w_up.T, B_w_down)
    return out.reshape(B, 1, D)
```

```python
import jax
import jax.numpy as jnp
import jax.experimental.pallas as pl
import jax.experimental.pallas.tpu as pltpu

B = 8
D = 512
H = 32
DH = 128
SK = 4096
W = min(4096, max(256, SK // 4))
F = 1376
EPS = 1e-05
G = 2
NG = B // G
FA = 1024
NT = (((1,), (1,)), ((), ()))
BF = jnp.bfloat16
F32 = jnp.float32

KV_PIECES = (
    (0, 0, 0, 64, 0), (1, 0, 64, 128, 1), (1, 0, 0, 64, 0), (1, 1, 896, 128, 0),
    (1, 1, 128, 128, 1), (1, 1, 0, 128, 0), (0, 1, 256, 128, 1), (0, 1, 384, 128, 0),
    (0, 0, 192, 128, 1), (0, 0, 320, 128, 1), (1, 0, 192, 128, 1), (0, 1, 128, 128, 1),
    (1, 0, 320, 128, 1), (1, 1, 256, 128, 1), (1, 1, 384, 128, 0), (0, 0, 448, 128, 1),
    (0, 1, 512, 128, 0), (0, 0, 576, 128, 1), (1, 0, 448, 128, 0), (1, 0, 576, 128, 1),
    (0, 1, 768, 128, 1), (0, 1, 640, 128, 1), (0, 0, 704, 128, 1), (1, 1, 640, 128, 1),
    (1, 1, 512, 128, 0), (0, 0, 832, 128, 0), (0, 1, 0, 128, 0), (0, 1, 896, 128, 0),
    (1, 0, 704, 128, 1), (1, 0, 832, 128, 0), (1, 1, 768, 128, 1), (0, 0, 64, 128, 1),
    (0, 0, 960, 64, 0), (1, 0, 960, 64, 0),
)


def _weight_pieces(nrows, cols, phase):
    if cols == 512:
        halves = [(16 * j, 16, 0, 512) for j in range(nrows // 16)]
    else:
        per = cols // 1024
        halves = [(8 * (j // per), 8, 1024 * (j % per), 1024) for j in range(nrows // 8 * per)]
    blocks = {}
    for j, half in enumerate(halves):
        blocks.setdefault((j + phase) // 2, []).append(half)
    out = []
    for m in sorted(blocks, key=lambda m: (m // 32, m % 4 // 2, m % 32 // 4, m % 2)):
        parts = blocks[m]
        if len(parts) == 2:
            (r0, n0, c0, w0), (r1, n1, c1, w1) = parts
            if c0 == c1:
                parts = [(r0, n0 + n1, c0, w0)]
            elif r0 == r1:
                parts = [(r0, n0, c0, w0 + w1)]
        out += [p + (1 - ((m ^ (m >> 1)) & 1),) for p in parts]
    return out


def _aligned(v, m):
    return v if isinstance(v, int) else pl.multiple_of(v, m)


def _layernorm(x):
    m = jnp.mean(x, axis=-1, keepdims=True)
    xc = x - m
    v = jnp.mean(xc * xc, axis=-1, keepdims=True)
    return xc / jnp.sqrt(v + EPS)


def _kernel(x_hbm, c_hbm, wmod_hbm, wq_hbm, k_hbm, v_hbm, wo_hbm, wg_hbm, wu_hbm, wd_hbm,
            out_ref,
            kbuf, vbuf, wmod_v, wq_v, wo_v, wg_v, wu_v, wd_v, x_v, c_v, q_s, o_s, sem):

    def wait_buf(buf, s):
        pltpu.make_async_copy(buf, buf, sem.at[s]).wait()

    def start_rows(src, dst, row0, nrows, s, phase=1, thread=None):
        for r, n, c, w, pr in _weight_pieces(nrows, src.shape[1], phase):
            if thread is None or pr == thread:
                win = (pl.ds(_aligned(row0 + r, 8), n), pl.ds(c, w))
                pltpu.make_async_copy(src.at[win], dst.at[win], sem.at[s]).start(priority=pr)

    def start_unit(i, g, has_k=True, has_v=True):
        for db, is_v, off, n, pr in KV_PIECES:
            b = g * G + db
            if not is_v and has_k:
                src, dst = k_hbm.at[b, i, pl.ds(SK - W + off, n), :], kbuf.at[b, pl.ds(off, n), :]
            elif is_v and has_v:
                src, dst = v_hbm.at[b, i - 1, pl.ds(SK - W + off, n), :], vbuf.at[b, pl.ds(off, n), :]
            elif not is_v:
                rows = pl.ds(b * 256 + off // 4, n // 4)
                src, dst = wo_hbm.at[rows, :], wo_v.at[rows, :]
            else:
                continue
            pltpu.make_async_copy(src, dst, sem.at[g]).start(priority=pr)

    cp_c = pltpu.make_async_copy(c_hbm, c_v, sem.at[0])
    cp_x = pltpu.make_async_copy(x_hbm, x_v, sem.at[0])
    cp_c.start()
    cp_x.start()
    rg = D // NG

    def wait_group(buf, j):
        wait_buf(buf.at[pl.ds(_aligned(j * rg, rg), rg), :], j)

    @pl.loop(0, NG)
    def _(j):
        start_rows(wmod_hbm, wmod_v, j * rg, rg, j, phase=0)

    cp_c.wait()
    cp_x.wait()

    @pl.loop(0, NG)
    def _(j):
        wait_group(wmod_v, j)
        start_rows(wq_hbm, wq_v, j * rg, rg, j)

    c = c_v[...].astype(F32)
    sc = (c * jax.nn.sigmoid(c)).astype(BF)
    mod = jnp.dot(sc, wmod_v[...], preferred_element_type=F32)
    sa, ca, ga, sb, cb, gb = [mod[:, i * D:(i + 1) * D] for i in range(6)]
    x = x_v[...].astype(F32)
    h = (_layernorm(x) * (1.0 + ca) + sa).astype(BF)

    @pl.loop(0, NG)
    def _(g):
        wait_group(wq_v, g)
        start_unit(0, g, has_v=False)

    qb = (jnp.dot(h, wq_v[...], preferred_element_type=F32) * (DH ** -0.5)).astype(BF)
    for i in range(H):
        q_s[i] = qb[:, i * DH:(i + 1) * DH]

    row_s = jax.lax.broadcasted_iota(jnp.int32, (B, W), 0)
    row_o = jax.lax.broadcasted_iota(jnp.int32, (B, DH), 0)

    def sweep(i, state, do_qk, do_pv, wait, refill):
        s = jnp.zeros((B, W), F32)
        o = jnp.zeros((B, DH), F32)
        qh = q_s[i] if do_qk else None
        for b in range(B):
            if b % G == 0:
                wait(b)
            if do_qk:
                s = jnp.where(row_s == b, jax.lax.dot_general(qh, kbuf[b], NT, preferred_element_type=F32), s)
            if do_pv:
                o = jnp.where(row_o == b, jnp.dot(state[0], vbuf[b], preferred_element_type=F32), o)
            if b % G == G - 1:
                refill(b // G)
        if do_pv:
            o_s[i - 1] = (o * state[1]).astype(BF)
        if not do_qk:
            return None
        p = jnp.exp(s - jnp.max(s, axis=-1, keepdims=True))
        return p.astype(BF), 1.0 / jnp.sum(p, axis=-1, keepdims=True)

    def wait_k(b):
        wait_buf(kbuf.at[pl.ds(b, G)], b // G)

    def wait_kv(b):
        wait_k(b)
        wait_buf(vbuf.at[pl.ds(b, G)], b // G)

    def wait_v_wo(b):
        wait_buf(vbuf.at[pl.ds(b, G)], b // G)
        wait_buf(wo_v.at[pl.ds(b * 256, 256 * G), :], b // G)

    tail = [(wo_hbm, wo_v, 2048, 1024, 0), (wo_hbm, wo_v, 3072, 1024, 1), (wg_hbm, wg_v, 0, F, 2),
            (wu_hbm, wu_v, 0, F, 3), (wd_hbm, wd_v, 0, FA, 0), (wd_hbm, wd_v, FA, F - FA, 1)]

    def tail_start(t, thread=None):
        src, dst, r0, n, s = tail[t]
        start_rows(src, dst, r0, n, s, thread=thread)

    def tail_wait(t):
        _, dst, r0, n, s = tail[t]
        wait_buf(dst.at[pl.ds(r0, n), :], s)

    st = sweep(0, None, True, False, wait_k, lambda g: start_unit(1, g))
    st = jax.lax.fori_loop(
        1, H - 1, lambda i, st: sweep(i, st, True, True, wait_kv, lambda g: start_unit(i + 1, g)), st)
    st = sweep(H - 1, st, True, True, wait_kv, lambda g: start_unit(H, g, has_k=False))
    sweep(H, st, False, True, wait_v_wo, tail_start)

    tail_wait(0)
    tail_wait(1)
    og = 4

    def obody(g, acc):
        for t in range(og):
            i = g * og + t
            acc = acc + jnp.dot(o_s[i], wo_v[pl.ds(pl.multiple_of(i * DH, DH), DH), :],
                                preferred_element_type=F32)
        return acc

    acc = jax.lax.fori_loop(0, H // og, obody, jnp.zeros((B, D), F32))
    tail_start(4, thread=1)
    x1 = x + ga * acc
    h2 = (_layernorm(x1) * (1.0 + cb) + sb).astype(BF)

    tail_wait(2)
    tail_start(5, thread=1)
    g = jax.lax.dot_general(h2, wg_v[...], NT, preferred_element_type=F32)
    tail_start(4, thread=0)
    tail_wait(3)
    tail_start(5, thread=0)
    u = jax.lax.dot_general(h2, wu_v[...], NT, preferred_element_type=F32)
    hm = (jax.nn.sigmoid(g) * u).astype(BF)
    for j in range(2):
        for t in range(4):
            o_s[j + 2 * t] = hm[:, j * 512 + t * 128:j * 512 + (t + 1) * 128]

    def dbody(j, y):
        @pl.when(j == 0)
        def _():
            tail_wait(4)

        for t in range(4):
            rows = pl.ds(pl.multiple_of(j * 512 + t * 128, 128), 128)
            y = y + jnp.dot(o_s[j + 2 * t], wd_v[rows, :], preferred_element_type=F32)
        return y

    y = jax.lax.fori_loop(0, 2, dbody, jnp.zeros((B, D), F32))
    tail_wait(5)
    y = y + jnp.dot(hm[:, FA:], wd_v[pl.ds(FA, F - FA), :], preferred_element_type=F32)
    out_ref[...] = (x1 + gb * y).astype(BF)


@jax.jit
def pallas_adaLN_cond__sliding_block_cached__glu_gated_glu__decode_kernel(
    A_x, A_k_cache, A_v_cache, A_wq, A_wo, B_x, B_w_gate, B_w_up, B_w_down, c, w_mod
):
    del B_x
    hbm = pl.BlockSpec(memory_space=pltpu.HBM)
    out = pl.pallas_call(
        _kernel,
        out_shape=jax.ShapeDtypeStruct((B, D), BF),
        in_specs=[hbm] * 10,
        out_specs=pl.BlockSpec(memory_space=pltpu.VMEM),
        scratch_shapes=[
            pltpu.VMEM((B, W, DH), BF),
            pltpu.VMEM((B, W, DH), BF),
            pltpu.VMEM((D, 6 * D), BF),
            pltpu.VMEM((D, H * DH), BF),
            pltpu.VMEM((H * DH, D), BF),
            pltpu.VMEM((F, D), BF),
            pltpu.VMEM((F, D), BF),
            pltpu.VMEM((F, D), BF),
            pltpu.VMEM((B, D), BF),
            pltpu.VMEM((B, D), BF),
            pltpu.VMEM((H, B, DH), BF),
            pltpu.VMEM((H, B, DH), BF),
            pltpu.SemaphoreType.DMA((NG,)),
        ],
        compiler_params=pltpu.CompilerParams(vmem_limit_bytes=64 * 1024 * 1024),
    )(A_x.reshape(B, D), c, w_mod, A_wq, A_k_cache, A_v_cache, A_wo,
      B_w_gate.T, B_w_up.T, B_w_down)
    return out.reshape(B, 1, D)
```

```python
import jax
import jax.numpy as jnp
import jax.experimental.pallas as pl
import jax.experimental.pallas.tpu as pltpu

B = 8
D = 512
H = 32
DH = 128
SK = 4096
W = min(4096, max(256, SK // 4))
F = 1376
EPS = 1e-05
G = 2
NG = B // G
FA = 768
NT = (((1,), (1,)), ((), ()))
BF = jnp.bfloat16
F32 = jnp.float32

KV_PIECES = (
    (0, 0, 0, 64, 0), (1, 0, 64, 128, 1), (1, 0, 0, 64, 0), (1, 1, 896, 128, 0),
    (1, 1, 128, 128, 1), (1, 1, 0, 128, 0), (0, 1, 256, 128, 1), (0, 1, 384, 128, 0),
    (0, 0, 192, 128, 1), (0, 0, 320, 128, 1), (1, 0, 192, 128, 1), (0, 1, 128, 128, 1),
    (1, 0, 320, 128, 1), (1, 1, 256, 128, 1), (1, 1, 384, 128, 0), (0, 0, 448, 128, 1),
    (0, 1, 512, 128, 0), (0, 0, 576, 128, 1), (1, 0, 448, 128, 0), (1, 0, 576, 128, 1),
    (0, 1, 768, 128, 1), (0, 1, 640, 128, 1), (0, 0, 704, 128, 1), (1, 1, 640, 128, 1),
    (1, 1, 512, 128, 0), (0, 0, 832, 128, 0), (0, 1, 0, 128, 0), (0, 1, 896, 128, 0),
    (1, 0, 704, 128, 1), (1, 0, 832, 128, 0), (1, 1, 768, 128, 1), (0, 0, 64, 128, 1),
    (0, 0, 960, 64, 0), (1, 0, 960, 64, 0),
)


def _weight_pieces(nrows, cols, phase):
    if cols == 512:
        halves = [(16 * j, 16, 0, 512) for j in range(nrows // 16)]
    else:
        per = cols // 1024
        halves = [(8 * (j // per), 8, 1024 * (j % per), 1024) for j in range(nrows // 8 * per)]
    blocks = {}
    for j, half in enumerate(halves):
        blocks.setdefault((j + phase) // 2, []).append(half)
    out = []
    for m in sorted(blocks, key=lambda m: (m // 32, m % 4 // 2, m % 32 // 4, m % 2)):
        parts = blocks[m]
        if len(parts) == 2:
            (r0, n0, c0, w0), (r1, n1, c1, w1) = parts
            if c0 == c1:
                parts = [(r0, n0 + n1, c0, w0)]
            elif r0 == r1:
                parts = [(r0, n0, c0, w0 + w1)]
        out += [p + (1 - ((m ^ (m >> 1)) & 1),) for p in parts]
    return out


def _aligned(v, m):
    return v if isinstance(v, int) else pl.multiple_of(v, m)


def _layernorm(x):
    m = jnp.mean(x, axis=-1, keepdims=True)
    xc = x - m
    v = jnp.mean(xc * xc, axis=-1, keepdims=True)
    return xc / jnp.sqrt(v + EPS)


def _kernel(x_hbm, c_hbm, wmod_hbm, wq_hbm, k_hbm, v_hbm, wo_hbm, wg_hbm, wu_hbm, wd_hbm,
            out_ref,
            kbuf, vbuf, wmod_v, wq_v, wo_v, wg_v, wu_v, wd_v, x_v, c_v, q_s, o_s, sem):

    def wait_buf(buf, s):
        pltpu.make_async_copy(buf, buf, sem.at[s]).wait()

    def start_rows(src, dst, row0, nrows, s, phase=1, thread=None):
        for r, n, c, w, pr in _weight_pieces(nrows, src.shape[1], phase):
            if thread is None or pr == thread:
                win = (pl.ds(_aligned(row0 + r, 8), n), pl.ds(c, w))
                pltpu.make_async_copy(src.at[win], dst.at[win], sem.at[s]).start(priority=pr)

    def start_unit(i, g, has_k=True, has_v=True):
        for db, is_v, off, n, pr in KV_PIECES:
            b = g * G + db
            if not is_v and has_k:
                src, dst = k_hbm.at[b, i, pl.ds(SK - W + off, n), :], kbuf.at[b, pl.ds(off, n), :]
            elif is_v and has_v:
                src, dst = v_hbm.at[b, i - 1, pl.ds(SK - W + off, n), :], vbuf.at[b, pl.ds(off, n), :]
            elif not is_v:
                rows = pl.ds(b * 256 + off // 4, n // 4)
                src, dst = wo_hbm.at[rows, :], wo_v.at[rows, :]
            else:
                continue
            pltpu.make_async_copy(src, dst, sem.at[g]).start(priority=pr)

    cp_c = pltpu.make_async_copy(c_hbm, c_v, sem.at[0])
    cp_x = pltpu.make_async_copy(x_hbm, x_v, sem.at[0])
    cp_c.start()
    cp_x.start()
    rg = D // NG

    def wait_group(buf, j):
        wait_buf(buf.at[pl.ds(_aligned(j * rg, rg), rg), :], j)

    @pl.loop(0, NG)
    def _(j):
        start_rows(wmod_hbm, wmod_v, j * rg, rg, j, phase=0)

    cp_c.wait()
    cp_x.wait()

    @pl.loop(0, NG)
    def _(j):
        wait_group(wmod_v, j)
        start_rows(wq_hbm, wq_v, j * rg, rg, j)

    c = c_v[...].astype(F32)
    sc = (c * jax.nn.sigmoid(c)).astype(BF)
    mod = jnp.dot(sc, wmod_v[...], preferred_element_type=F32)
    sa, ca, ga, sb, cb, gb = [mod[:, i * D:(i + 1) * D] for i in range(6)]
    x = x_v[...].astype(F32)
    h = (_layernorm(x) * (1.0 + ca) + sa).astype(BF)

    @pl.loop(0, NG)
    def _(g):
        wait_group(wq_v, g)
        start_unit(0, g, has_v=False)

    qb = (jnp.dot(h, wq_v[...], preferred_element_type=F32) * (DH ** -0.5)).astype(BF)
    for i in range(H):
        q_s[i] = qb[:, i * DH:(i + 1) * DH]

    row_s = jax.lax.broadcasted_iota(jnp.int32, (B, W), 0)
    row_o = jax.lax.broadcasted_iota(jnp.int32, (B, DH), 0)

    def sweep(i, state, do_qk, do_pv, wait, refill):
        s = jnp.zeros((B, W), F32)
        o = jnp.zeros((B, DH), F32)
        qh = q_s[i] if do_qk else None
        for b in range(B):
            if b % G == 0:
                wait(b)
            if do_qk:
                s = jnp.where(row_s == b, jax.lax.dot_general(qh, kbuf[b], NT, preferred_element_type=F32), s)
            if do_pv:
                o = jnp.where(row_o == b, jnp.dot(state[0], vbuf[b], preferred_element_type=F32), o)
            if b % G == G - 1:
                refill(b // G)
        if do_pv:
            o_s[i - 1] = (o * state[1]).astype(BF)
        if not do_qk:
            return None
        p = jnp.exp(s - jnp.max(s, axis=-1, keepdims=True))
        return p.astype(BF), 1.0 / jnp.sum(p, axis=-1, keepdims=True)

    def wait_k(b):
        wait_buf(kbuf.at[pl.ds(b, G)], b // G)

    def wait_kv(b):
        wait_k(b)
        wait_buf(vbuf.at[pl.ds(b, G)], b // G)

    def wait_v_wo(b):
        wait_buf(vbuf.at[pl.ds(b, G)], b // G)
        wait_buf(wo_v.at[pl.ds(b * 256, 256 * G), :], b // G)

    tail = [(wo_hbm, wo_v, 2048, 1024, 0), (wo_hbm, wo_v, 3072, 1024, 1), (wg_hbm, wg_v, 0, F, 2),
            (wu_hbm, wu_v, 0, F, 3), (wd_hbm, wd_v, 0, FA, 0), (wd_hbm, wd_v, FA, F - FA, 1)]

    def tail_start(t, thread=None):
        src, dst, r0, n, s = tail[t]
        start_rows(src, dst, r0, n, s, thread=thread)

    def tail_wait(t):
        _, dst, r0, n, s = tail[t]
        wait_buf(dst.at[pl.ds(r0, n), :], s)

    st = sweep(0, None, True, False, wait_k, lambda g: start_unit(1, g))
    st = jax.lax.fori_loop(
        1, H - 1, lambda i, st: sweep(i, st, True, True, wait_kv, lambda g: start_unit(i + 1, g)), st)
    st = sweep(H - 1, st, True, True, wait_kv, lambda g: start_unit(H, g, has_k=False))
    sweep(H, st, False, True, wait_v_wo, tail_start)

    tail_wait(0)
    tail_wait(1)
    og = 4

    def obody(g, acc):
        for t in range(og):
            i = g * og + t
            acc = acc + jnp.dot(o_s[i], wo_v[pl.ds(pl.multiple_of(i * DH, DH), DH), :],
                                preferred_element_type=F32)
        return acc

    acc = jax.lax.fori_loop(0, H // og, obody, jnp.zeros((B, D), F32))
    tail_start(4, thread=1)
    x1 = x + ga * acc
    h2 = (_layernorm(x1) * (1.0 + cb) + sb).astype(BF)

    tail_wait(2)
    tail_start(5, thread=1)
    g = jax.lax.dot_general(h2, wg_v[...], NT, preferred_element_type=F32)
    tail_start(4, thread=0)
    tail_wait(3)
    tail_start(5, thread=0)
    u = jax.lax.dot_general(h2, wu_v[...], NT, preferred_element_type=F32)
    hm = (jax.nn.sigmoid(g) * u).astype(BF)
    for j in range(2):
        for t in range(3):
            o_s[j + 2 * t] = hm[:, j * 384 + t * 128:j * 384 + (t + 1) * 128]

    def dbody(j, y):
        @pl.when(j == 0)
        def _():
            tail_wait(4)

        for t in range(3):
            rows = pl.ds(pl.multiple_of(j * 384 + t * 128, 128), 128)
            y = y + jnp.dot(o_s[j + 2 * t], wd_v[rows, :], preferred_element_type=F32)
        return y

    y = jax.lax.fori_loop(0, 2, dbody, jnp.zeros((B, D), F32))
    tail_wait(5)
    y = y + jnp.dot(hm[:, FA:], wd_v[pl.ds(FA, F - FA), :], preferred_element_type=F32)
    out_ref[...] = (x1 + gb * y).astype(BF)


@jax.jit
def pallas_adaLN_cond__sliding_block_cached__glu_gated_glu__decode_kernel(
    A_x, A_k_cache, A_v_cache, A_wq, A_wo, B_x, B_w_gate, B_w_up, B_w_down, c, w_mod
):
    del B_x
    hbm = pl.BlockSpec(memory_space=pltpu.HBM)
    out = pl.pallas_call(
        _kernel,
        out_shape=jax.ShapeDtypeStruct((B, D), BF),
        in_specs=[hbm] * 10,
        out_specs=pl.BlockSpec(memory_space=pltpu.VMEM),
        scratch_shapes=[
            pltpu.VMEM((B, W, DH), BF),
            pltpu.VMEM((B, W, DH), BF),
            pltpu.VMEM((D, 6 * D), BF),
            pltpu.VMEM((D, H * DH), BF),
            pltpu.VMEM((H * DH, D), BF),
            pltpu.VMEM((F, D), BF),
            pltpu.VMEM((F, D), BF),
            pltpu.VMEM((F, D), BF),
            pltpu.VMEM((B, D), BF),
            pltpu.VMEM((B, D), BF),
            pltpu.VMEM((H, B, DH), BF),
            pltpu.VMEM((H, B, DH), BF),
            pltpu.SemaphoreType.DMA((NG,)),
        ],
        compiler_params=pltpu.CompilerParams(vmem_limit_bytes=64 * 1024 * 1024),
    )(A_x.reshape(B, D), c, w_mod, A_wq, A_k_cache, A_v_cache, A_wo,
      B_w_gate.T, B_w_up.T, B_w_down)
    return out.reshape(B, 1, D)
```
